```python
import jax
import jax.numpy as jnp

def _softmax(x, axis=-1):
    return jax.nn.softmax(x, axis=axis)
def _gelu(x):
    return jax.nn.gelu(x, approximate=True)
def _silu(x):
    return jax.nn.silu(x)
def _sigmoid(x):
    return jax.nn.sigmoid(x)
def _layernorm(x, axis=-1, eps=1e-5):
    m = jnp.mean(x, axis=axis, keepdims=True)
    v = jnp.var(x, axis=axis, keepdims=True)
    return (x - m) / jnp.sqrt(v + eps)
def _scatter_add(tgt, idx, src, axis=0):
    return tgt.at[idx].add(src)
def _segment_sum(src, seg, n):
    return jax.ops.segment_sum(src, seg, n)
class _Rng:
    def __init__(self, key):
        self._k = key
    def _next(self):
        self._k, sub = jax.random.split(self._k)
        return sub
    def normal(self, shape):
        return jax.random.normal(self._next(), shape, dtype=jnp.bfloat16)
    def randint(self, lo, hi, shape):
        return jax.random.randint(self._next(), shape, lo, hi, dtype=jnp.int32)
    def uniform(self, shape, lo=0.0, hi=1.0):
        return jax.random.uniform(self._next(), shape, jnp.bfloat16, lo, hi)
    def permutation(self, n):
        return jax.random.permutation(self._next(), n)


kernel_name = 'standalone__batchnorm__sampling'

def setup_inputs():
    _rng = _Rng(jax.random.key(int.from_bytes(__import__("os").urandom(4), "little")))
    _w = (lambda a: (lambda t: t.astype(jnp.bfloat16) if jnp.issubdtype(t.dtype, jnp.floating) else t)(jnp.asarray(a)))
    B, S, C = 1024, 32, 576
    K = 3
    return {
        "x": _w((lambda *s: _rng.normal(s) * 0.05)(B, S, C)),
        "w": _w((lambda *s: _rng.normal(s) * 0.05)(K, C, C) * (1.0 / (K * C) ** 0.5)),
        "mean": _w((lambda *s: _rng.normal(s) * 0.05)(C) * 0.1),
        "var": _w(jnp.abs((lambda *s: _rng.normal(s) * 0.05)(C)) + 0.5),
        "g": _w((lambda *s: _rng.normal(s) * 0.05)(C) + 1.0),
        "b": _w((lambda *s: _rng.normal(s) * 0.05)(C) * 0.1),
    }

def reference(x, w, mean, var, g, b):
    K = 3
    P = K // 2
    S = x.shape[1]
    xp = jnp.pad(x, ((0, 0), (P, P), (0, 0)))
    y = sum(jnp.einsum('bsc,cd->bsd', xp[:, k:k + S, :], w[k]) for k in range(K))
    inv_std = 1.0 / jnp.sqrt(var + 1e-5)
    y = (y - mean) * (g * inv_std) + b
    return _silu(y)
```

```python
import jax, jax.numpy as jnp
from jax import lax
from jax.experimental import pallas as pl
from jax.experimental.pallas import tpu as pltpu
BN = 128
A = 1.5
Bq = 1.0 / A
F32, BF16 = jnp.float32, jnp.bfloat16

def _g_rows():
    a, b = A, Bq
    pts = [0.0, a, -a, b, -b]
    rows = []
    for i, p in enumerate(pts):
        f = 1.0
        for j, q in enumerate(pts):
            if j != i:
                f *= (p - q)
        rows.append([1.0 / f, p / f, p * p / f])
    rows.append([0.0, 0.0, 1.0])
    return rows

def kern(x_ref, w_ref, mean_ref, var_ref, g_ref, b_ref, o_ref, gt_ref, bias_ref):
    S, C, bn = x_ref.shape
    @pl.when(pl.program_id(0) == 0)
    def _():
        sc = g_ref[...].astype(F32) * lax.rsqrt(var_ref[...].astype(F32) + 1e-5)
        bias = b_ref[...].astype(F32) - mean_ref[...].astype(F32) * sc
        bias_ref[...] = jnp.broadcast_to(bias * 0.5, (128, C)).T
        w0, w1, w2 = [w_ref[k].astype(F32) * (sc * 0.5) for k in range(3)]
        for i, r in enumerate(_g_rows()):
            gi = r[0] * w0 + r[1] * w1 + r[2] * w2
            gt_ref[i] = gi.T.astype(BF16)
    a, b = A, Bq
    a2, b2 = a * a, b * b
    bias = bias_ref[...]
    if bn > 128:
        bias = jnp.concatenate([bias] * (bn // 128), axis=1)
    for j in range(S // 4):
        d = []
        for r in range(6):
            s = 4 * j - 1 + r
            d.append(x_ref[s].astype(F32) if 0 <= s < S else None)
        d0, d1, d2, d3, d4, d5 = d
        c2 = a2 + b2
        u0 = d4 - c2 * d2 if d0 is None else d0 - c2 * d2 + d4
        u5 = d1 - c2 * d3 if d5 is None else d1 - c2 * d3 + d5
        ea, oa = d4 - b2 * d2, a * d3 - b * d1
        eb, ob = d4 - a2 * d2, b * d3 - a * d1
        us = [u0, ea + oa, ea - oa, eb + ob, eb - ob, u5]
        m = [jnp.dot(gt_ref[i], us[i].astype(BF16), preferred_element_type=F32) for i in range(6)]
        sa, da = m[1] + m[2], m[1] - m[2]
        sb, db = m[3] + m[4], m[3] - m[4]
        ys = [m[0] + sa + sb, a * da + b * db, a2 * sa + b2 * sb, (a2 * a) * da + (b2 * b) * db + m[5]]
        for r in range(4):
            h = ys[r] + bias
            o_ref[4 * j + r] = (h * jnp.tanh(h) + h).astype(BF16)

@jax.jit
def pallas_standalone__batchnorm__sampling_kernel(x, w, mean, var, g, b):
    B, S, C = x.shape
    xt = jnp.transpose(x, (1, 2, 0))
    vec = pl.BlockSpec((1, C), lambda i: (0, 0))
    out = pl.pallas_call(kern,
        grid=(B // BN,),
        in_specs=[pl.BlockSpec((S, C, BN), lambda i: (0, 0, i)), pl.BlockSpec((3, C, C), lambda i: (0, 0, 0)), vec, vec, vec, vec],
        out_specs=pl.BlockSpec((S, C, BN), lambda i: (0, 0, i)),
        out_shape=jax.ShapeDtypeStruct((S, C, B), x.dtype),
        scratch_shapes=[pltpu.VMEM((6, C, C), BF16), pltpu.VMEM((C, 128), F32)],
        compiler_params=pltpu.CompilerParams(dimension_semantics=("arbitrary",), vmem_limit_bytes=100*1024*1024),
    )(xt, w, mean.reshape(1, C), var.reshape(1, C), g.reshape(1, C), b.reshape(1, C))
    return jnp.transpose(out, (2, 0, 1))
```

```python
import jax, jax.numpy as jnp
from jax import lax
from jax.experimental import pallas as pl
from jax.experimental.pallas import tpu as pltpu
BN = 128
F32, BF16 = jnp.float32, jnp.bfloat16
TILES = [6, 6, 4, 6, 6, 4]
PTS = {4: (1.5, 1.0 / 1.5), 6: (1.0, 2.0, 0.5)}

def _mul(c, v):
    return v if c == 1.0 else c * v

def _lin(terms):
    acc = None
    for c, v in terms:
        if v is None or c == 0.0:
            continue
        if acc is None:
            acc = v if c == 1.0 else c * v
        elif c < 0:
            acc = acc - _mul(-c, v)
        else:
            acc = acc + _mul(c, v)
    return acc

def _polymul(p, q):
    r = [0.0] * (len(p) + len(q) - 1)
    for i, a in enumerate(p):
        for j, b in enumerate(q):
            r[i + j] += a * b
    return r

def _even_poly(ps):
    r = [1.0]
    for p in ps:
        r = _polymul(r, [-p * p, 1.0])
    return r

def u_transform(d, ps):
    full = _even_poly(ps)
    us = [_lin([(c, d[2 * i]) for i, c in enumerate(full)][::-1])]
    for k, p in enumerate(ps):
        N = _even_poly([q for i, q in enumerate(ps) if i != k])
        e = _lin([(c, d[2 * i + 2]) for i, c in enumerate(N)][::-1])
        o = _lin([(p * c, d[2 * i + 1]) for i, c in enumerate(N)][::-1])
        us += [e + o, e - o]
    us.append(_lin([(c, d[2 * i + 1]) for i, c in enumerate(full)][::-1]))
    return us

def g_transform(w0, w1, w2, ps):
    f0 = 1.0
    for p in ps:
        f0 *= -p * p
    gs = [_mul(1.0 / f0, w0)]
    for k, p in enumerate(ps):
        f = 2.0 * p * p
        for i, q in enumerate(ps):
            if i != k:
                f *= p * p - q * q
        e, o = (1.0 / f) * w0 + (p * p / f) * w2, (p / f) * w1
        gs += [e + o, e - o]
    gs.append(w2)
    return gs

def y_transform(m, ps):
    nout = 2 * len(ps)
    sd = [(m[1 + 2 * k] + m[2 + 2 * k], m[1 + 2 * k] - m[2 + 2 * k]) for k in range(len(ps))]
    ys = []
    for r in range(nout):
        terms = [(p ** r, sd[k][r % 2]) for k, p in enumerate(ps)]
        if r == 0:
            terms = [(1.0, m[0])] + terms
        if r == nout - 1:
            terms = terms + [(1.0, m[-1])]
        ys.append(_lin(terms))
    return ys

def _kernel(x_hbm, w_hbm, mean_ref, var_ref, g_ref, b_ref, o_hbm, gt_ref, bias_ref, wbuf, xbuf, obuf, wsem, xsem, osem):
    S, C, B = x_hbm.shape
    n = pl.program_id(0)
    nsteps = pl.num_programs(0)
    slot = n % 2
    sizes = sorted(set(TILES))
    goff = {}
    o = 0
    for m in sizes:
        goff[m] = o
        o += m + 2
    def xcopy(nn, sl):
        return pltpu.make_async_copy(x_hbm.at[:, :, pl.ds(nn * BN, BN)], xbuf.at[sl], xsem.at[sl])
    def ocopy(nn, sl, s0, m):
        return pltpu.make_async_copy(obuf.at[sl, pl.ds(s0, m)], o_hbm.at[pl.ds(s0, m), :, pl.ds(nn * BN, BN)], osem.at[sl])
    def owait(sl):
        pltpu.make_async_copy(obuf.at[sl], obuf.at[sl], osem.at[sl]).wait()

    @pl.when(n == 0)
    def _():
        wc = pltpu.make_async_copy(w_hbm, wbuf, wsem)
        wc.start()
        xcopy(0, 0).start()
        sc = g_ref[...].astype(F32).reshape(1, C) * lax.rsqrt(var_ref[...].astype(F32).reshape(1, C) + 1e-5)
        bias = b_ref[...].astype(F32).reshape(1, C) - mean_ref[...].astype(F32).reshape(1, C) * sc
        bias_ref[...] = jnp.broadcast_to(bias * 0.5, (128, C)).T
        sccol = jnp.broadcast_to(sc * 0.5, (128, C)).T
        wc.wait()
        for c0 in range(0, C, 128):
            cw = min(128, C - c0)
            scc = sccol[c0:c0 + cw]
            for kt, k0 in enumerate(range(0, C, 128)):
                kw = min(128, C - k0)
                w0, w1, w2 = [wbuf[k, k0:k0 + kw, c0:c0 + cw].T.astype(F32) * scc[:, :kw] for k in range(3)]
                for m in sizes:
                    for i, gi in enumerate(g_transform(w0, w1, w2, PTS[m])):
                        gt_ref[goff[m] + i, kt, c0:c0 + cw, :kw] = gi.astype(BF16)

    @pl.when(n + 1 < nsteps)
    def _():
        xcopy(n + 1, 1 - slot).start()

    @pl.when(n >= 2)
    def _():
        owait(slot)

    xcopy(n, slot).wait()
    bias = bias_ref[...]
    s0 = 0
    for m in TILES:
        d = [xbuf[slot, s].astype(F32) if 0 <= s < S else None for s in range(s0 - 1, s0 + m + 1)]
        us = u_transform(d, PTS[m])
        ms = []
        for i, u in enumerate(us):
            u = u.astype(BF16)
            acc = None
            for kt, k0 in enumerate(range(0, C, 128)):
                kw = min(128, C - k0)
                p = jnp.dot(gt_ref[goff[m] + i, kt, :, :kw], u[k0:k0 + kw], preferred_element_type=F32)
                acc = p if acc is None else acc + p
            ms.append(acc)
        ys = y_transform(ms, PTS[m])
        for r in range(m):
            h = ys[r] + bias
            obuf[slot, s0 + r] = (h * jnp.tanh(h) + h).astype(BF16)
        ocopy(n, slot, s0, m).start()
        s0 += m

    @pl.when(n == nsteps - 1)
    def _():
        owait(1 - slot)
        owait(slot)

@jax.jit
def pallas_standalone__batchnorm__sampling_kernel(x, w, mean, var, g, b):
    B, S, C = x.shape
    xt = jnp.transpose(x, (1, 2, 0))
    vec = pl.BlockSpec((C,), lambda i: (0,))
    hbm = pl.BlockSpec(memory_space=pl.ANY)
    ng = sum(m + 2 for m in set(TILES))
    out = pl.pallas_call(_kernel,
        grid=(B // BN,),
        in_specs=[hbm, hbm, vec, vec, vec, vec],
        out_specs=hbm,
        out_shape=jax.ShapeDtypeStruct((S, C, B), x.dtype),
        scratch_shapes=[pltpu.VMEM((ng, pl.cdiv(C, 128), C, 128), BF16), pltpu.VMEM((C, 128), F32), pltpu.VMEM((3, C, C), BF16),
                        pltpu.VMEM((2, S, C, BN), BF16), pltpu.VMEM((2, S, C, BN), BF16),
                        pltpu.SemaphoreType.DMA(()), pltpu.SemaphoreType.DMA((2,)), pltpu.SemaphoreType.DMA((2,))],
        compiler_params=pltpu.CompilerParams(dimension_semantics=("arbitrary",), vmem_limit_bytes=100*1024*1024),
    )(xt, w, mean, var, g, b)
    return jnp.transpose(out, (2, 0, 1))
```
